```python
import os as _os
_os.environ.setdefault("JAX_PLATFORMS", "cpu")
import jax
import jax.numpy as jnp

def _softmax(x, axis=-1):
    return jax.nn.softmax(x, axis=axis)
def _gelu(x):
    return jax.nn.gelu(x, approximate=True)
def _silu(x):
    return jax.nn.silu(x)
def _sigmoid(x):
    return jax.nn.sigmoid(x)
def _layernorm(x, axis=-1, eps=1e-5):
    m = jnp.mean(x, axis=axis, keepdims=True)
    v = jnp.var(x, axis=axis, keepdims=True)
    return (x - m) / jnp.sqrt(v + eps)
def _scatter_add(tgt, idx, src, axis=0):
    return tgt.at[idx].add(src)
def _segment_sum(src, seg, n):
    return jax.ops.segment_sum(src, seg, n)
class _Rng:
    def __init__(self, key):
        self._k = key
    def _next(self):
        self._k, sub = jax.random.split(self._k)
        return sub
    def normal(self, shape):
        return jax.random.normal(self._next(), shape, dtype=jnp.bfloat16)
    def randint(self, lo, hi, shape):
        return jax.random.randint(self._next(), shape, lo, hi, dtype=jnp.int32)
    def uniform(self, shape, lo=0.0, hi=1.0):
        return jax.random.uniform(self._next(), shape, jnp.bfloat16, lo, hi)
    def permutation(self, n):
        return jax.random.permutation(self._next(), n)


kernel_name = 'standalone__gqa_softmax__decode'

def setup_inputs():
    _rng = _Rng(jax.random.key(int.from_bytes(__import__("os").urandom(4), "little")))
    _w = (lambda a: (lambda t: t.astype(jnp.bfloat16) if jnp.issubdtype(t.dtype, jnp.floating) else t)(jnp.asarray(a)))
    B, Hq, Hkv, Sq, Sk, D = 2, 32, 32, 1, 8192, 128
    return {
        "q": _w((lambda *s: _rng.normal(s) * 0.8)(B, Hq, Sq, D)),
        "k": _w((lambda *s: _rng.normal(s) * 0.8)(B, Hkv, Sk, D)),
        "v": _w((lambda *s: _rng.normal(s) * 0.05)(B, Hkv, Sk, D)),
    }

def reference(q, k, v):
    B, Hq, Sq, D = q.shape
    Hkv = k.shape[1]
    rep = Hq // Hkv
    k = jnp.repeat(k, rep, axis=1)
    v = jnp.repeat(v, rep, axis=1)
    scale = D ** -0.5
    scores = jnp.einsum("bhqd,bhkd->bhqk", q, k) * scale
    p = _softmax(scores, axis=-1)
    return jnp.einsum("bhqk,bhkd->bhqd", p, v)
```

```python
import math

import jax
import jax.numpy as jnp
from jax import lax
import jax.experimental.pallas as pl
import jax.experimental.pallas.tpu as pltpu

_CHUNK = 256
_GROUP = 4
_HI_SLOTS = 16
_LO_SLOTS = 8
_ROWS = 8


@jax.jit
def pallas_standalone__gqa_softmax__decode_kernel(
    q: jax.Array,
    k: jax.Array,
    v: jax.Array,
):
    B, H, _, D = q.shape
    S = k.shape[2]
    s, g1, n0, m1, M = _CHUNK, _GROUP, _HI_SLOTS, _LO_SLOTS, _ROWS
    NH = B * H
    R = NH * S
    G = g1 * s
    C = S // s
    GH = S // G
    half = S // 2
    TA = C // 2
    GA = GH // 2
    NT = NH * C
    NG = NT // g1
    c_exp = (D ** -0.5) * math.log2(math.e)

    def kern(q_hbm, k_hbm, v_hbm, o_hbm, b0, b1, s_buf, q_raw, q_f32, o_f32, o_bf, sem0, sem1, semq):
        def p0_copy(src, row, slot):
            return pltpu.make_async_copy(src.at[pl.ds(pl.multiple_of(row, s), s)], b0.at[slot], sem0.at[slot])

        def p1_copy(src, row, slot):
            return pltpu.make_async_copy(src.at[pl.ds(pl.multiple_of(row, G), G)], b1.at[slot], sem1.at[slot])

        def p0_wait(slot):
            pltpu.make_async_copy(b0.at[slot], b0.at[slot], sem0.at[slot]).wait()

        def p1_wait(slot):
            pltpu.make_async_copy(b1.at[slot], b1.at[slot], sem1.at[slot]).wait()

        def p0_start_static(b):
            if b < TA:
                p0_copy(k_hbm, half + b * s, b % n0).start(priority=0)
            else:
                p0_copy(v_hbm, (b - TA) * s, b % n0).start(priority=0)

        def p1_start_static(a):
            if a < GA:
                p1_copy(k_hbm, a * G, a % m1).start(priority=1)
            else:
                p1_copy(k_hbm, (a + GA) * G, a % m1).start(priority=1)

        def p0_start(b, phase):
            slot = lax.rem(b, n0)
            if phase == "a":
                @pl.when(b < TA)
                def _():
                    p0_copy(k_hbm, half + b * s, slot).start(priority=0)

                @pl.when(b >= TA)
                def _():
                    p0_copy(v_hbm, (b - TA) * s, slot).start(priority=0)
            else:
                @pl.when(b < NT)
                def _():
                    p0_copy(v_hbm, (b - TA) * s, slot).start(priority=0)

        def p1_start(a, phase):
            slot = lax.rem(a, m1)
            if phase == "a":
                @pl.when(a < GA)
                def _():
                    p1_copy(k_hbm, a * G, slot).start(priority=1)

                @pl.when(a >= GA)
                def _():
                    p1_copy(k_hbm, (a + GA) * G, slot).start(priority=1)
            else:
                if phase == "b":
                    @pl.when(a < NG - GA)
                    def _():
                        p1_copy(k_hbm, (a + GA) * G, slot).start(priority=1)

                @pl.when(jnp.logical_and(a >= NG - GA, a < NG))
                def _():
                    p1_copy(v_hbm, a * G, slot).start(priority=1)

        p1_start_static(0)
        qc = pltpu.make_async_copy(q_hbm, q_raw, semq)
        qc.start(priority=0)
        p0_start_static(0)
        for a in range(1, m1 - 1):
            p1_start_static(a)
        for b in range(1, n0 - 1):
            p0_start_static(b)
        qc.wait()
        q_f32[...] = q_raw[...].astype(jnp.float32)

        def load_q(h):
            return jnp.broadcast_to(q_f32[pl.ds(h, 1), :], (M, D)).astype(jnp.bfloat16)

        def qk(qv, kc):
            return lax.dot_general(qv, kc, (((1,), (1,)), ((), ())), preferred_element_type=jnp.float32)

        def tile_max(m, sc):
            for i in range(s // 128):
                m = jnp.maximum(m, sc[:, i * 128:(i + 1) * 128])
            return m

        def probs(sc, m, l):
            ps = []
            for i in range(s // 128):
                p = jnp.exp2((sc[:, i * 128:(i + 1) * 128] - m) * c_exp)
                l = l + p
                ps.append(p)
            return jnp.concatenate(ps, axis=1).astype(jnp.bfloat16), l

        def row_max(m):
            return jnp.broadcast_to(jnp.max(m, axis=1, keepdims=True), m.shape)

        neg = jnp.full((M, 128), -jnp.inf, jnp.float32)
        zero = jnp.zeros((M, 128), jnp.float32)

        q0 = load_q(0)

        def body_a(a, m):
            slot1 = lax.rem(a, m1)
            p1_wait(slot1)
            p1_start(a + (m1 - 1), "a")
            for u in range(g1):
                t = a * g1 + u
                slot0 = lax.rem(t, n0)
                p0_wait(slot0)
                p0_start(t + (n0 - 1), "a")
                s1 = qk(q0, b1[slot1, pl.ds(u * s, s), :])
                s0 = qk(q0, b0[slot0])
                s_buf[t] = s1
                s_buf[t + TA] = s0
                m = tile_max(tile_max(m, s1), s0)
            return m

        m_run = lax.fori_loop(0, GA, body_a, neg)

        def body_h(h, m_run):
            m = row_max(m_run)
            qv = load_q(h + 1)

            def body_g(jg, carry):
                m_new, l, acc = carry
                a = GA + h * GH + jg
                slot1 = lax.rem(a, m1)
                p1_wait(slot1)
                p1_start(a + (m1 - 1), "b")
                for u in range(g1):
                    t = a * g1 + u
                    j = jg * g1 + u
                    slot0 = lax.rem(t, n0)
                    p0_wait(slot0)
                    p0_start(t + (n0 - 1), "b")
                    p, l = probs(s_buf[j], m, l)
                    sc = qk(qv, b1[slot1, pl.ds(u * s, s), :])
                    acc = acc + jnp.dot(p, b0[slot0], preferred_element_type=jnp.float32)
                    s_buf[j] = sc
                    m_new = tile_max(m_new, sc)
                return m_new, l, acc

            m_new, l, acc = lax.fori_loop(0, GH, body_g, (neg, zero, zero))
            o = acc / jnp.sum(l, axis=1, keepdims=True)
            o_f32[pl.ds(h, 1), :] = o[0:1]
            return m_new

        m_run = lax.fori_loop(0, NH - 1, body_h, m_run)

        m = row_max(m_run)

        def body_c(jg, carry):
            l, acc = carry
            a = NG - GA + jg
            slot1 = lax.rem(a, m1)
            p1_wait(slot1)
            if m1 - 1 < GA:
                p1_start(a + (m1 - 1), "c")
            for u in range(g1):
                t = a * g1 + u
                j = jg * g1 + u
                slot0 = lax.rem(t, n0)
                p0_wait(slot0)
                if n0 - 1 < TA:
                    p0_start(t + (n0 - 1), "c")
                pa, l = probs(s_buf[j], m, l)
                pb, l = probs(s_buf[j + TA], m, l)
                acc = acc + jnp.dot(pa, b0[slot0], preferred_element_type=jnp.float32)
                acc = acc + jnp.dot(pb, b1[slot1, pl.ds(u * s, s), :], preferred_element_type=jnp.float32)
            return l, acc

        l, acc = lax.fori_loop(0, GA, body_c, (zero, zero))
        o = acc / jnp.sum(l, axis=1, keepdims=True)
        o_f32[pl.ds(NH - 1, 1), :] = o[0:1]
        o_bf[...] = o_f32[...].astype(o_bf.dtype)
        oc = pltpu.make_async_copy(o_bf, o_hbm, semq)
        oc.start()
        oc.wait()

    out = pl.pallas_call(
        kern,
        in_specs=[pl.BlockSpec(memory_space=pl.ANY)] * 3,
        out_specs=pl.BlockSpec(memory_space=pl.ANY),
        out_shape=jax.ShapeDtypeStruct((NH, D), q.dtype),
        scratch_shapes=[
            pltpu.VMEM((n0, s, D), k.dtype),
            pltpu.VMEM((m1, G, D), k.dtype),
            pltpu.VMEM((C, M, s), jnp.float32),
            pltpu.VMEM((NH, D), q.dtype),
            pltpu.VMEM((NH, D), jnp.float32),
            pltpu.VMEM((NH, D), jnp.float32),
            pltpu.VMEM((NH, D), q.dtype),
            pltpu.SemaphoreType.DMA((n0,)),
            pltpu.SemaphoreType.DMA((m1,)),
            pltpu.SemaphoreType.DMA(()),
        ],
        compiler_params=pltpu.CompilerParams(
            vmem_limit_bytes=64 << 20,
            disable_bounds_checks=True,
            disable_semaphore_checks=True,
        ),
    )(q.reshape(NH, D), k.reshape(R, D), v.reshape(R, D))
    return out.reshape(q.shape)
```

```python
import functools
import math

import jax
import jax.numpy as jnp
from jax import lax
import jax.experimental.pallas as pl
import jax.experimental.pallas.tpu as pltpu

_LANES = 128
_ROWS = 8
_BLOCK = 1024
_K_PIECES = (256, 256, 256, 256)
_V_PIECES = (248, 248, 248, 280)
_K_SHIFT, _V_SHIFT = 192, 176
_K_AHEAD, _V_AHEAD = 5, 11
_K_SLOTS, _V_SLOTS = 8, 16


def _pieces(lengths, shift, kind):
    out, offset = [], 0
    for n in lengths:
        lo, hi = offset, offset + n
        if kind == "first":
            lo = max(lo, _BLOCK - shift)
        if kind == "last":
            hi = min(hi, _BLOCK - shift)
        if hi > lo:
            out.append((lo, hi - lo))
        offset += n
    return out


def _split_rows(rows, parts):
    out = [rows // parts // 8 * 8] * parts
    out[-1] += rows - sum(out)
    return out


def _kernel(q_hbm, k_hbm, v_hbm, o_hbm,
            ring, q_f32, o_f32, o_out, k_sems, v_sems, qo_sem, *, seq_len):
    heads, dim = q_hbm.shape
    blocks = k_hbm.shape[0] // _BLOCK
    per_head = seq_len // _BLOCK
    log2_per_head = per_head.bit_length() - 1
    scale_log2e = dim ** -0.5 * math.log2(math.e)

    k_stream = (k_hbm, 0, k_sems, _K_SLOTS, _K_SHIFT, _K_PIECES, 0)
    v_stream = (v_hbm, _K_SLOTS, v_sems, _V_SLOTS, _V_SHIFT, _V_PIECES, 1)

    def copy(stream, cycle, offset, rows):
        src, base, sems, slots, shift, _, priority = stream
        slot = (cycle + 1) & (slots - 1)
        row = cycle * _BLOCK + shift + offset
        if not isinstance(row, int):
            row = pl.multiple_of(row, 8)
        if not isinstance(offset, int):
            offset = pl.multiple_of(offset, 8)
        dma = pltpu.make_async_copy(
            src.at[pl.ds(row, rows)], ring.at[base + slot, pl.ds(offset, rows)], sems.at[slot])
        return dma, priority

    def copies(stream, cycle, kind):
        return [copy(stream, cycle, o, n) for o, n in _pieces(stream[5], stream[4], kind)]

    def start(k_copies, v_copies):
        for j in range(max(len(k_copies), len(v_copies))):
            for group in (k_copies, v_copies):
                if j < len(group):
                    dma, priority = group[j]
                    dma.start(priority=priority)

    def wait(stream, cycle, kind):
        _, base, sems, slots, shift, lengths, _ = stream
        slot = (cycle + 1) & (slots - 1)
        pieces = _pieces(lengths, shift, kind)
        filled = ring.at[base + slot, pl.ds(pieces[0][0], sum(n for _, n in pieces))]
        pltpu.make_async_copy(filled, filled, sems.at[slot]).wait()

    def load_block(stream, block):
        _, base, _, slots, shift, _, _ = stream
        lo = ring[base + (block & (slots - 1)), pl.ds(_BLOCK - shift, shift), :]
        hi = ring[base + ((block + 1) & (slots - 1)), pl.ds(0, _BLOCK - shift), :]
        return jnp.concatenate([lo, hi], axis=0)

    lead = _V_AHEAD - _K_AHEAD
    tail_groups = _split_rows(_BLOCK - _V_SHIFT, lead + 1)

    def v_tail(group, rows):
        out, offset = [], group * tail_groups[0]
        for n in _split_rows(rows, len(_K_PIECES)):
            out.append(copy(v_stream, blocks - 1, offset, n))
            offset = offset + n
        return out

    def request(step):
        k_cycle, v_cycle = step + _K_AHEAD, step + _V_AHEAD

        @pl.when(v_cycle < blocks - 1)
        def _():
            start(copies(k_stream, k_cycle, "full"), copies(v_stream, v_cycle, "full"))

        @pl.when(jnp.logical_and(v_cycle >= blocks - 1, k_cycle < blocks - 1))
        def _():
            start(copies(k_stream, k_cycle, "full"),
                  v_tail(v_cycle - (blocks - 1), tail_groups[0]))

        @pl.when(k_cycle == blocks - 1)
        def _():
            start(copies(k_stream, blocks - 1, "last"), v_tail(lead, tail_groups[-1]))

    def softmax_terms(block, m, l):
        new_head = (block & (per_head - 1)) == 0
        q_row = q_f32[pl.ds(block >> log2_per_head, 1), :]
        q_rows = jnp.broadcast_to(q_row, (_ROWS, dim)).astype(ring.dtype)
        s = lax.dot_general(q_rows, load_block(k_stream, block), (((1,), (1,)), ((), ())),
                            preferred_element_type=jnp.float32)
        tiles = [s[:, t:t + _LANES] for t in range(0, _BLOCK, _LANES)]
        block_max = jnp.max(functools.reduce(jnp.maximum, tiles), axis=1, keepdims=True)
        m_old = jnp.where(new_head, -jnp.inf, m)
        m_new = jnp.maximum(m_old, block_max)
        m_sub = jnp.where(m_new == -jnp.inf, 0.0, m_new)
        alpha = jnp.exp2((m_old - m_sub) * scale_log2e)
        p = [jnp.exp2((t - m_sub) * scale_log2e) for t in tiles]
        l = jnp.where(new_head, 0.0, l * alpha) + functools.reduce(jnp.add, p)
        return m_new, l, alpha, jnp.concatenate(p, axis=1).astype(ring.dtype)

    def accumulate(block, l, alpha, p, acc):
        new_head = (block & (per_head - 1)) == 0
        inv_l = 1.0 / jnp.sum(l, axis=1, keepdims=True)
        acc = jnp.where(new_head, 0.0, acc * alpha) + jnp.dot(
            p, load_block(v_stream, block), preferred_element_type=jnp.float32)
        o_f32[pl.ds(block >> log2_per_head, 1), :] = (acc * inv_l)[0:1]
        return acc

    q_raw = ring.at[0, pl.ds(0, heads)]
    q_copy = pltpu.make_async_copy(q_hbm, q_raw, qo_sem)
    start([], copies(v_stream, -1, "first"))
    q_copy.start()
    start(copies(k_stream, -1, "first"), [])
    for c in range(lead):
        start([], copies(v_stream, c, "full"))
    for c in range(_K_AHEAD):
        start(copies(k_stream, c, "full"), copies(v_stream, c + lead, "full"))
    q_copy.wait()
    q_f32[...] = q_raw[...].astype(jnp.float32)
    wait(k_stream, -1, "first")
    wait(v_stream, -1, "first")

    o_f32[pl.ds(0, _ROWS), :] = jnp.zeros((_ROWS, dim), jnp.float32)
    zero = o_f32[pl.ds(0, _ROWS), :]

    def step(i, carry):
        m, l, alpha, p, acc = carry

        @pl.when(i + 1 < blocks - 1)
        def _():
            wait(k_stream, i + 1, "full")

        @pl.when(i + 1 == blocks - 1)
        def _():
            wait(k_stream, i + 1, "last")

        wait(v_stream, i, "full")
        terms = softmax_terms(i + 1, m, l)
        acc = accumulate(i, l, alpha, p, acc)
        request(i)
        return terms + (acc,)

    wait(k_stream, 0, "full")
    carry = softmax_terms(0, zero, zero) + (zero,)
    _, l, alpha, p, acc = lax.fori_loop(0, blocks - 1, step, carry)
    wait(v_stream, blocks - 1, "last")
    accumulate(blocks - 1, l, alpha, p, acc)

    o_out[...] = o_f32[...].astype(o_out.dtype)
    o_copy = pltpu.make_async_copy(o_out, o_hbm, qo_sem)
    o_copy.start()
    o_copy.wait()


@jax.jit
def pallas_standalone__gqa_softmax__decode_kernel(
    q: jax.Array,
    k: jax.Array,
    v: jax.Array,
):
    batch, q_heads, q_len, dim = q.shape
    seq_len = k.shape[2]
    heads = batch * q_heads
    per_head = seq_len // _BLOCK
    assert q_len == 1 and dim == _LANES and k.shape[1] == q_heads and v.shape == k.shape
    assert q.dtype == k.dtype == v.dtype
    assert seq_len % _BLOCK == 0 and per_head & (per_head - 1) == 0
    assert _ROWS <= heads <= _BLOCK - _K_SHIFT and heads * per_head > _V_AHEAD
    assert _K_SLOTS >= _K_AHEAD + 2 and _V_SLOTS >= _V_AHEAD + 2

    out = pl.pallas_call(
        functools.partial(_kernel, seq_len=seq_len),
        in_specs=[pl.BlockSpec(memory_space=pl.ANY)] * 3,
        out_specs=pl.BlockSpec(memory_space=pl.ANY),
        out_shape=jax.ShapeDtypeStruct((heads, dim), q.dtype),
        scratch_shapes=[
            pltpu.VMEM((_K_SLOTS + _V_SLOTS, _BLOCK, dim), k.dtype),
            pltpu.VMEM((heads, dim), jnp.float32),
            pltpu.VMEM((heads, dim), jnp.float32),
            pltpu.VMEM((heads, dim), q.dtype),
            pltpu.SemaphoreType.DMA((_K_SLOTS,)),
            pltpu.SemaphoreType.DMA((_V_SLOTS,)),
            pltpu.SemaphoreType.DMA(()),
        ],
        compiler_params=pltpu.CompilerParams(
            disable_bounds_checks=True,
            disable_semaphore_checks=True,
        ),
    )(q.reshape(heads, dim),
      k.reshape(heads * seq_len, dim),
      v.reshape(heads * seq_len, dim))
    return out.reshape(q.shape)
```
